```python
import jax
import jax.numpy as jnp

def _softmax(x, axis=-1):
    return jax.nn.softmax(x, axis=axis)
def _gelu(x):
    return jax.nn.gelu(x, approximate=True)
def _silu(x):
    return jax.nn.silu(x)
def _sigmoid(x):
    return jax.nn.sigmoid(x)
def _layernorm(x, axis=-1, eps=1e-5):
    m = jnp.mean(x, axis=axis, keepdims=True)
    v = jnp.var(x, axis=axis, keepdims=True)
    return (x - m) / jnp.sqrt(v + eps)
def _scatter_add(tgt, idx, src, axis=0):
    return tgt.at[idx].add(src)
def _segment_sum(src, seg, n):
    return jax.ops.segment_sum(src, seg, n)
class _Rng:
    def __init__(self, key):
        self._k = key
    def _next(self):
        self._k, sub = jax.random.split(self._k)
        return sub
    def normal(self, shape):
        return jax.random.normal(self._next(), shape, dtype=jnp.bfloat16)
    def randint(self, lo, hi, shape):
        return jax.random.randint(self._next(), shape, lo, hi, dtype=jnp.int32)
    def uniform(self, shape, lo=0.0, hi=1.0):
        return jax.random.uniform(self._next(), shape, jnp.bfloat16, lo, hi)
    def permutation(self, n):
        return jax.random.permutation(self._next(), n)


kernel_name = 'parallel_sum__linear_attn_block__moe_arch_mod__prompt'

def setup_inputs():
    _rng = _Rng(jax.random.key(int.from_bytes(__import__("os").urandom(4), "little")))
    _w = (lambda a: (lambda t: t.astype(jnp.bfloat16) if jnp.issubdtype(t.dtype, jnp.floating) else t)(jnp.asarray(a)))
    def _A_setup():
        B, S, D = 1, 2048, 1024
        return {
            "x": _w((lambda *s: _rng.normal(s) * 0.05)(B, S, D)),
            "wqkv": _w((lambda *s: _rng.normal(s) * 0.05)(D, 3 * D)),
            "wo": _w((lambda *s: _rng.normal(s) * 0.05)(D, D)),
        }
    _A_in = _A_setup()

    def _B_setup():
        B, S, D, F, C = 1, 2048, 1024, 3584, 1
        return {
            "x": _w((lambda *s: _rng.normal(s) * 0.05)(B, S, D)),
            "w_r": _w((lambda *s: _rng.normal(s) * 0.05)(D)),
            "w_gate": _w((lambda *s: _rng.normal(s) * 0.05)(D, F)),
            "w_up": _w((lambda *s: _rng.normal(s) * 0.05)(D, F)),
            "w_down": _w((lambda *s: _rng.normal(s) * 0.05)(F, D)),
        }
    _B_in = _B_setup()

    return {
        "A_x": _A_in["x"],
        "A_wqkv": _A_in["wqkv"],
        "A_wo": _A_in["wo"],
        "B_x": _B_in["x"],
        "B_w_r": _B_in["w_r"],
        "B_w_gate": _B_in["w_gate"],
        "B_w_up": _B_in["w_up"],
        "B_w_down": _B_in["w_down"],
    }

def reference(A_x, A_wqkv, A_wo, B_x, B_w_r, B_w_gate, B_w_up, B_w_down):
    def _A_ref(x, wqkv, wo):
        B, S, D = x.shape
        H = 32; Dh = D // H
        qkv = (lambda x, *d: x.transpose(*d))((x @ wqkv).reshape(B, S, 3, H, Dh), 2, 0, 3, 1, 4)
        q, k, v = qkv[0], qkv[1], qkv[2]
        phi = lambda t: jnp.where(t > 0, t + 1, jnp.exp(t)) + 1e-6
        pq, pk = phi(q), phi(k)
        kv = jnp.einsum("bhsd,bhse->bhde", pk, v)
        z = jnp.einsum("bhsd->bhd", pk)
        num = jnp.einsum("bhqd,bhde->bhqe", pq, kv)
        den = jnp.einsum("bhqd,bhd->bhq", pq, z)[..., None] + 1e-6
        o = num / den
        return (lambda x, *d: x.transpose(*d))(o, 0, 2, 1, 3).reshape(B, S, D) @ wo

    def _B_ref(x, w_r, w_gate, w_up, w_down):
        B, S, D = x.shape
        C = 1
        r = x @ w_r
        idx = jnp.argsort(-r, axis=-1)[:, :C]
        idx_e = jnp.repeat(idx.reshape(B, C, 1), D, axis=2)
        x_sel = jnp.take_along_axis(x, idx_e, axis=1)
        g = _silu(x_sel @ w_gate)
        u = x_sel @ w_up
        y = (g * u) @ w_down
        r_sel = _sigmoid(jnp.take_along_axis(r, idx, axis=1))
        y = y * r_sel.reshape(B, C, 1)
        b_off = (jnp.arange(B) * S).reshape(B, 1)
        flat_idx = (idx + b_off).reshape(B * C)
        zero = (x * 0.0).reshape(B * S, D)
        upd = _scatter_add(zero, flat_idx, y.reshape(B * C, D), axis=0)
        return x + upd.reshape(B, S, D)

    x = A_x
    xn = _layernorm(x, axis=-1)
    return x + _A_ref(xn, A_wqkv, A_wo) + _B_ref(xn, B_w_r, B_w_gate, B_w_up, B_w_down)
```

```python
import functools
import numpy as np
import jax
import jax.numpy as jnp
from jax import lax
import jax.experimental.pallas as pl
import jax.experimental.pallas.tpu as pltpu

S, D, F, H, DH = 2048, 1024, 3584, 32, 32
BM = 256
NB = S // BM
f32, bf16 = jnp.float32, jnp.bfloat16


def _phi(t):
    return jnp.where(t > 0, t + 1.0, jnp.exp(t)) + 1e-6


def _rnd(t):
    return t.astype(bf16).astype(f32)


def kernel(x_hbm, wqkv_hbm, wo_hbm, wr_hbm, wg_hbm, wu_hbm, wd_hbm, o_hbm,
           x_v, wqkv_v, wo_v, wr_v, wg_v, wu_v, wd_v, xn_v, pq_v, o_v,
           kv_v, z_v, m_v, zbd_v, sem_x, sem_w, sem_o):
    def xcopy(i):
        return pltpu.make_async_copy(x_hbm.at[0, pl.ds(i * BM, BM)], x_v.at[pl.ds(i * BM, BM)], sem_x.at[i])

    def ocopy(i):
        return pltpu.make_async_copy(o_v.at[pl.ds(i * BM, BM)], o_hbm.at[0, pl.ds(i * BM, BM)], sem_o.at[i])

    c_wr = pltpu.make_async_copy(wr_hbm, wr_v, sem_w.at[0])
    c_wqkv = pltpu.make_async_copy(wqkv_hbm, wqkv_v, sem_w.at[1])
    c_wo = pltpu.make_async_copy(wo_hbm, wo_v, sem_w.at[2])
    c_wg = pltpu.make_async_copy(wg_hbm, wg_v, sem_w.at[3])
    c_wu = pltpu.make_async_copy(wu_hbm, wu_v, sem_w.at[4])
    c_wd = pltpu.make_async_copy(wd_hbm, wd_v, sem_w.at[5])
    xcopy(0).start()
    c_wr.start()
    c_wqkv.start()
    for i in range(1, NB):
        xcopy(i).start()
    c_wo.start()
    c_wg.start()
    c_wu.start()
    c_wd.start()

    kv_v[...] = jnp.zeros_like(kv_v)
    z_v[...] = jnp.zeros_like(z_v)
    c_wr.wait()
    wr = wr_v[...].astype(f32)
    c_wqkv.wait()

    def p1(i, carry):
        bval, bidx = carry
        r0 = pl.multiple_of(i * BM, BM)
        xcopy(i).wait()
        x = x_v[pl.ds(r0, BM), :].astype(f32)
        mean = jnp.sum(x, axis=1, keepdims=True) * (1.0 / D)
        xc = x - mean
        var = jnp.sum(xc * xc, axis=1, keepdims=True) * (1.0 / D)
        m_b = _rnd(mean)
        s_b = _rnd(jnp.sqrt(_rnd(_rnd(var) + _rnd(jnp.float32(1e-5)))))
        xn = ((x - m_b) / s_b).astype(bf16)
        xn_v[pl.ds(r0, BM), :] = xn
        r = jnp.sum(xn.astype(f32) * wr, axis=1, keepdims=True)
        rb = _rnd(r)
        mx = jnp.max(rb, axis=0, keepdims=True)
        rows = (lax.broadcasted_iota(jnp.int32, (BM, 1), 0) + r0).astype(f32)
        ci = jnp.min(jnp.where(rb == mx, rows, 1e9), axis=0, keepdims=True)
        upd = mx > bval
        bval = jnp.where(upd, mx, bval)
        bidx = jnp.where(upd, ci, bidx)
        q = jnp.dot(xn, wqkv_v[:, 0:D], preferred_element_type=f32)
        pq_v[pl.ds(r0, BM), :] = _phi(q).astype(bf16)
        k = jnp.dot(xn, wqkv_v[:, D:2 * D], preferred_element_type=f32)
        pk = _phi(k).astype(bf16)
        v = jnp.dot(xn, wqkv_v[:, 2 * D:3 * D], preferred_element_type=f32).astype(bf16)
        z_v[...] += jnp.sum(pk.astype(f32), axis=0, keepdims=True)
        for j in range(8):
            kv_v[j] += lax.dot_general(pk[:, j * 128:(j + 1) * 128], v[:, j * 128:(j + 1) * 128],
                                       (((0,), (0,)), ((), ())), preferred_element_type=f32)
        return bval, bidx

    bval, bidx = lax.fori_loop(0, NB, p1, (jnp.full((1, 1), -jnp.inf, f32), jnp.zeros((1, 1), f32)))

    ri = lax.broadcasted_iota(jnp.int32, (128, 128), 0) // DH
    ci_ = lax.broadcasted_iota(jnp.int32, (128, 128), 1) // DH
    bd = ri == ci_
    c_wo.wait()
    zb = z_v[...].astype(bf16).astype(f32)
    for j in range(8):
        kvj = jnp.where(bd, kv_v[j], 0.0).astype(bf16)
        m_v[pl.ds(j * 128, 128), :] = jnp.dot(kvj, wo_v[pl.ds(j * 128, 128), :], preferred_element_type=f32).astype(bf16)
        zrow = jnp.broadcast_to(zb[:, j * 128:(j + 1) * 128], (128, 128))
        zcol = zrow.T
        zbd_v[j] = jnp.where(bd, zcol, 0.0).astype(bf16)

    idx = jnp.max(bidx).astype(jnp.int32)
    base = pl.multiple_of((idx // 16) * 16, 16)
    tile = xn_v[pl.ds(base, 16), :].astype(f32)
    trow = lax.broadcasted_iota(jnp.int32, (16, D), 0) + base
    xs = jnp.where(trow == idx, tile, 0.0).astype(bf16)
    c_wg.wait()
    g = jnp.dot(xs, wg_v[...], preferred_element_type=f32)
    c_wu.wait()
    u = jnp.dot(xs, wu_v[...], preferred_element_type=f32)
    hh = (g * jax.nn.sigmoid(g) * u).astype(bf16)
    c_wd.wait()
    y = jnp.dot(hh, wd_v[...], preferred_element_type=f32)
    y = jnp.sum(y, axis=0, keepdims=True) * jax.nn.sigmoid(bval)

    def p2(i, _):
        r0 = pl.multiple_of(i * BM, BM)
        pq = pq_v[pl.ds(r0, BM), :]
        dens = []
        for j in range(8):
            dens.append(jnp.dot(pq[:, j * 128:(j + 1) * 128], zbd_v[j], preferred_element_type=f32))
        den = jnp.concatenate(dens, axis=1) + 1e-6
        pqn = (pq.astype(f32) / den).astype(bf16)
        a = jnp.dot(pqn, m_v[...], preferred_element_type=f32)
        x = x_v[pl.ds(r0, BM), :].astype(f32)
        xn = xn_v[pl.ds(r0, BM), :].astype(f32)
        rows = lax.broadcasted_iota(jnp.int32, (BM, D), 0) + r0
        res = x + a + xn + jnp.where(rows == idx, y, 0.0)
        o_v[pl.ds(r0, BM), :] = res.astype(bf16)
        ocopy(i).start()
        return 0

    lax.fori_loop(0, NB, p2, 0)
    for i in range(NB):
        ocopy(i).wait()


@jax.jit
def pallas_parallel_sum__linear_attn_block__moe_arch_mod__prompt_kernel(
        A_x, A_wqkv, A_wo, B_x, B_w_r, B_w_gate, B_w_up, B_w_down):
    del B_x
    any_spec = pl.BlockSpec(memory_space=pl.ANY)
    return pl.pallas_call(
        kernel,
        out_shape=jax.ShapeDtypeStruct((1, S, D), bf16),
        in_specs=[any_spec] * 7,
        out_specs=any_spec,
        scratch_shapes=[
            pltpu.VMEM((S, D), bf16), pltpu.VMEM((D, 3 * D), bf16), pltpu.VMEM((D, D), bf16),
            pltpu.VMEM((1, D), bf16), pltpu.VMEM((D, F), bf16), pltpu.VMEM((D, F), bf16),
            pltpu.VMEM((F, D), bf16), pltpu.VMEM((S, D), bf16), pltpu.VMEM((S, D), bf16),
            pltpu.VMEM((S, D), bf16),
            pltpu.VMEM((8, 128, 128), f32), pltpu.VMEM((1, D), f32), pltpu.VMEM((D, D), bf16),
            pltpu.VMEM((8, 128, 128), bf16),
            pltpu.SemaphoreType.DMA((NB,)), pltpu.SemaphoreType.DMA((6,)), pltpu.SemaphoreType.DMA((NB,)),
        ],
        compiler_params=pltpu.CompilerParams(vmem_limit_bytes=100 * 1024 * 1024),
        name="psum_la_mod",
    )(A_x, A_wqkv, A_wo, B_w_r.reshape(1, D), B_w_gate, B_w_up, B_w_down)
```

```python
import functools
import numpy as np
import jax
import jax.numpy as jnp
from jax import lax
import jax.experimental.pallas as pl
import jax.experimental.pallas.tpu as pltpu

S, D, F, H, DH = 2048, 1024, 3584, 32, 32
BT = 512
NB = S // BT
TQ = BT // 4
FQ = D // 4
MCK = 256
MCQ = 256
MCG = 256
MO = 128
f32, bf16, i32, u32 = jnp.float32, jnp.bfloat16, jnp.int32, jnp.uint32
LAG = 2
KSPAN = 0.95

UA = [{0: 1, 3: 1}, {2: 1, 3: 1}, {0: 1}, {3: 1}, {0: 1, 1: 1}, {2: 1, 0: -1}, {1: 1, 3: -1}]
UB = [{0: 1, 3: 1}, {0: 1}, {1: 1, 3: -1}, {2: 1, 0: -1}, {3: 1}, {0: 1, 1: 1}, {2: 1, 3: 1}]
WC = {0: {0: 1, 3: 1, 4: -1, 6: 1}, 1: {2: 1, 4: 1}, 2: {1: 1, 3: 1}, 3: {0: 1, 1: -1, 2: 1, 5: 1}}
PI = [0, 2, 6, 5, 3, 4, 1]
PORDER = [2, 4, 1, 3, 0, 6, 5]


def _lin(terms):
    acc = None
    for s, v in terms:
        if acc is None:
            acc = v if s > 0 else -v
        else:
            acc = acc + v if s > 0 else acc - v
    return acc


def st_ops(blocks, lvl, U):
    if lvl == 0:
        return [blocks[(0, 0)]]
    h = 2 ** (lvl - 1)
    quad = {q: {(r, c): blocks[(r + (q // 2) * h, c + (q % 2) * h)] for r in range(h) for c in range(h)}
            for q in range(4)}
    out = []
    for u in U:
        sub = {(r, c): _lin([(s, quad[q][(r, c)]) for q, s in sorted(u.items(), key=lambda t: -t[1])])
               for r in range(h) for c in range(h)}
        out += st_ops(sub, lvl - 1, U)
    return out


def st_combine(getp, lvl, base=0):
    if lvl == 0:
        return {(0, 0): getp(base)}
    h = 2 ** (lvl - 1)
    acc = {q: None for q in range(4)}
    for p in PORDER:
        m = st_combine(getp, lvl - 1, base * 7 + p)
        for q in range(4):
            if p in WC[q]:
                s = WC[q][p]
                if acc[q] is None:
                    acc[q] = (s, m)
                else:
                    s0, a = acc[q]
                    if s0 > 0:
                        acc[q] = (1, {k: (a[k] + m[k] if s > 0 else a[k] - m[k]) for k in m})
                    else:
                        assert s > 0
                        acc[q] = (1, {k: m[k] - a[k] for k in m})
    res = {}
    for q in range(4):
        assert acc[q][0] > 0
        for (r, c), v in acc[q][1].items():
            res[(r + (q // 2) * h, c + (q % 2) * h)] = v
    return res


def _dot(a, b):
    return jnp.dot(a, b, preferred_element_type=f32)


def _dot_nt(a, b):
    return lax.dot_general(a, b, (((1,), (1,)), ((), ())), preferred_element_type=f32)


def _phi(t):
    return jnp.where(t > 0, t + 1.0, jnp.exp(t)) + 1e-6


def _rnd(t):
    return t.astype(bf16).astype(f32)


def _rsum(v):
    return jnp.broadcast_to(jnp.sum(v, axis=1, keepdims=True), (v.shape[0], 128))


def _rcp(t):
    return pltpu.reciprocal(t, approx=False, full_range=False)


def _tiles(v):
    return [v[:, t * 128:(t + 1) * 128] for t in range(v.shape[1] // 128)]


def _layernorm_tiles(xt):
    mean = _rsum(functools.reduce(lambda a, b: a + b, xt)) * (1.0 / D)
    var = _rsum(functools.reduce(lambda a, b: a + b, [(t - mean) * (t - mean) for t in xt])) * (1.0 / D)
    m_b = _rnd(mean)
    s_b = _rnd(jnp.sqrt(_rnd(_rnd(var) + EPS_B)))
    rs = _rcp(s_b)
    return [(t - m_b) * rs for t in xt]


import contextlib
scope = lambda n: contextlib.nullcontext()
EPS_B = float(np.float32(1.0013580322265625e-05))


def _b16(v):
    return pltpu.bitcast(v, bf16)


def kernel(x_hbm, wqkv_hbm, wo_hbm, wr_hbm, wg_hbm, wu_hbm, wd_hbm, o_hbm, *scr):
    it = iter(scr)
    take = lambda n: [next(it) for _ in range(n)]
    x_v, wq_v, wk_v, wv_v, wo_v, wr_v, wg_v, wu_v, wd_v = take(9)
    o_v = take(NB)
    xn_t, wot_v = take(2)
    wt_v = take(2)
    sem_x, sem_w, sem_o, sem_g, sem_u, sem_d = take(6)
    NF = F // 128
    FG = 4

    def xcopy(b):
        return pltpu.make_async_copy(x_hbm.at[0, pl.ds(b * BT, BT)], x_v.at[pl.ds(b * BT, BT)], sem_x.at[b])

    def ocopy(b):
        return pltpu.make_async_copy(o_v[b], o_hbm.at[0, pl.ds(b * BT, BT)], sem_o.at[b])

    def wk_copy(m, c):
        return pltpu.make_async_copy(wqkv_hbm.at[:, pl.ds(D + c * FQ + m * 128, 128)],
                                     wk_v.at[:, pl.ds(c * FQ + m * 128, 128)], sem_w.at[8 + m * 4 + c])

    c_wr = pltpu.make_async_copy(wr_hbm, wr_v, sem_w.at[0])
    c_wv = pltpu.make_async_copy(wqkv_hbm.at[:, pl.ds(2 * D, D)], wv_v, sem_w.at[2])
    c_wo = pltpu.make_async_copy(wo_hbm, wo_v, sem_w.at[3])
    c_wq = pltpu.make_async_copy(wqkv_hbm.at[:, pl.ds(0, D)], wq_v, sem_w.at[4])
    c_wg = [pltpu.make_async_copy(wg_hbm.at[:, pl.ds(n * 128, 128)], wg_v.at[n], sem_g.at[n]) for n in range(NF)]
    c_wu = [pltpu.make_async_copy(wu_hbm.at[:, pl.ds(n * 128, 128)], wu_v.at[n], sem_u.at[n]) for n in range(NF)]
    c_wd = [pltpu.make_async_copy(wd_hbm.at[:, pl.ds(n * 128, 128)], wd_v.at[n], sem_d.at[n]) for n in range(8)]
    c_x0 = [pltpu.make_async_copy(x_hbm.at[0, pl.ds(q * TQ, TQ)], x_v.at[pl.ds(q * TQ, TQ)], sem_x.at[NB + q])
            for q in range(4)]
    c_x0[0].start()
    c_wr.start()
    for q in range(1, 4):
        c_x0[q].start()
    for m in range(2):
        for c in range(4):
            wk_copy(m, c).start()

    def start_ffn_copies():
        for c in c_wd:
            c.start()
        for n in range(NF):
            c_wg[n].start()
            c_wu[n].start()

    late = list(c_wd)
    for n in range(NF):
        late += [c_wg[n], c_wu[n]]
    st = {}
    c_wr.wait()
    wr16 = jnp.broadcast_to(wr_v[...].reshape(1, D), (16, D))
    xn_u = xn_t.bitcast(u32)
    stats = {}
    best = {}

    def xl(b, g, t):
        r0 = b * BT + g * 16
        return x_v[r0:r0 + 16, t * 128:(t + 1) * 128].astype(f32)

    def ln_a(b, g):
        s_ = xl(b, g, 0)
        for t in range(1, 8):
            s_ = s_ + xl(b, g, t)
        mean = _rsum(s_) * (1.0 / D)
        stats[("m", b, g)] = mean
        return pltpu.bitcast(mean[8:16, :], u32)

    def ln_b(b, g):
        mean = stats.pop(("m", b, g))
        q = None
        for t in range(8):
            e = xl(b, g, t) - mean
            q = e * e if q is None else q + e * e
        var = _rsum(q) * (1.0 / D)
        m_b = _rnd(mean)
        s_b = _rnd(jnp.sqrt(_rnd(_rnd(var) + EPS_B)))
        rs = _rcp(s_b)
        if "fmask" not in st:
            sb = s_b[0:8, :]
            st["fmask"] = sb < 0.0
            st["z"] = [jnp.max(jnp.where(sb < -float(k), 1.0, 0.0)).astype(i32) for k in range(2)]
        stats[(b, g)] = (m_b, rs)
        return pltpu.bitcast(rs[8:16, :], u32)

    def ln_c(b, g):
        r0 = b * BT + g * 16
        m_b, rs = stats.pop((b, g))
        for t in range(8):
            xn_t[t, r0:r0 + 16, :] = ((xl(b, g, t) - m_b) * rs).astype(bf16)

    def r_part(b, tt, t, pieces):
        t0 = b * BT + tt * 128
        ru = xn_u[t, pl.ds(t0 // 2, 64), :]
        k = 0
        for fn, buf in pieces:
            tok = fn()
            pend.append((len(hosted) + LAG, tok if buf is None else anchor(buf)))
        hosted.append(0)
        last = tt == 3 and t == 7
        while pend and (last or pend[0][0] <= len(hosted)):
            tok = pend.pop(0)[1]
            hd = jnp.where(st["fmask"], tok, ru[8 * k:8 * k + 8, :])
            ru = jnp.concatenate(([ru[:8 * k, :]] if k else []) + [hd] + ([ru[8 * k + 8:, :]] if k < 7 else []), axis=0)
            k = min(k + 1, 7)
        d = _dot_nt(wr16[:, t * 128:(t + 1) * 128], _b16(ru))[0:8, :]
        acc = d if t == 0 else racc.pop() + d
        if t < 7:
            racc.append(acc)
            return
        rr = _rnd(acc)
        if t0 == 0:
            best["row0"] = rr[0:1, 0:1]
        kb = pltpu.bitcast(jnp.where(rr == rr, rr, -jnp.inf), i32)
        kb = kb ^ ((kb >> 31) & 0x7FFFFFFF)
        kb = (kb & (-65536)) | (65535 - t0 - lax.broadcasted_iota(i32, (8, 128), 1))
        best["k"] = kb if "k" not in best else jnp.maximum(best["k"], kb)

    pend = []
    hosted = []
    racc = []

    def wt_piece(w_ref, m, r, c):
        for kt in range(2):
            t = w_ref[r * FQ + kt * 128:r * FQ + (kt + 1) * 128, c * FQ + m * 128:c * FQ + (m + 1) * 128]
            wt_v[m][(r * 4 + c) * 2 + kt] = t.astype(f32).T

    def wot_piece(j, t):
        v = wo_v[j * 128:(j + 1) * 128, t * 128:(t + 1) * 128].astype(f32).T
        wot_v[j, t * 128:(t + 1) * 128, :] = v.astype(bf16)

    def anchor(buf):
        idx = (st["z"][1],) + (0,) * (len(buf.shape) - 3) + (pl.ds(0, 8), pl.ds(0, 128))
        if buf.dtype == bf16:
            return buf.bitcast(u32)[idx]
        return pltpu.bitcast(buf[idx], u32)

    class Weave:
        def __init__(self, jobs, nslots):
            self.i = 0
            self.todo = [((j * nslots) // len(jobs), fn) for j, fn in enumerate(jobs)] if jobs else []

        def __call__(self, v):
            while self.todo and self.todo[0][0] <= self.i:
                self.todo.pop(0)[1]()
            self.i += 1
            return v

    P = functools.partial

    def f_ln(b):
        out = []
        for j in range(34):
            if j < 32:
                out.append((P(ln_a, b, j), None))
            if 1 <= j < 33:
                out.append((P(ln_b, b, j - 1), None))
            if j >= 2:
                out.append((P(ln_c, b, j - 2), xn_t))
        return out

    def f_wt(w_ref, m):
        return [(P(wt_piece, w_ref, m, r, c), wt_v[m]) for c in range(4) for r in range(4)]

    def split(lst, n):
        return [lst[i * len(lst) // n:(i + 1) * len(lst) // n] for i in range(n)]

    def make_w_ops(m):
        blocks = {(r, c): jnp.concatenate([wt_v[m][(r * 4 + c) * 2 + kt] for kt in range(2)], axis=1)
                  for r in range(4) for c in range(4)}
        return [o.astype(bf16) for o in st_ops(blocks, 2, UB)]

    s_ops = [None] * NB

    def make_s_ops(b):
        blocks = {(r, c): jnp.concatenate([xn_t[2 * c + kt, b * BT + r * TQ:b * BT + (r + 1) * TQ, :].astype(f32)
                                           for kt in range(2)], axis=1) for r in range(4) for c in range(4)}
        s_ops[b] = [o.astype(bf16) for o in st_ops(blocks, 2, UA)]

    def proj(wops, b, weave):
        return st_combine(lambda p: weave(_dot_nt(wops[p], s_ops[b][p])), 2)

    for q in range(4):
        c_x0[q].wait()
        for g in range(8 * q, 8 * q + 8):
            ln_a(0, g)
        for g in range(8 * q, 8 * q + 8):
            ln_b(0, g)
        for g in range(8 * q, 8 * q + 8):
            ln_c(0, g)
    for c in range(4):
        wk_copy(0, c).wait()
        for r in range(4):
            wt_piece(wk_v, 0, r, c)
    for c in range(4):
        wk_copy(1, c).wait()
    xcopy(1).start()
    wkt = [make_w_ops(0), None]

    g_acc = {}
    z_acc = {}
    for b in range(NB):
      with scope("A%d" % b):
        if 1 <= b < NB - 1:
            xcopy(b + 1).wait()
        if b == NB - 1:
            c_wq.wait()
            c_wo.wait()
            c_wv.wait()
        make_s_ops(b)
        if b + 1 < NB:
            lnp = f_ln(b + 1)
            per = [[] for _ in range(32)]
            first = 11 if b == 0 else 0
            for j, pc in enumerate(lnp):
                per[first + (j * (32 - first - LAG)) // len(lnp)].append(pc)
            if b == 0:
                for j, pc in enumerate(f_wt(wk_v, 1)):
                    per[j // 4].append(pc)
        else:
            fl = f_wt(wq_v, 0) + f_wt(wq_v, 1) + [(P(wot_piece, j, t), wot_v) for j in range(8) for t in range(8)]
            per = [[] for _ in range(32)]
            for j, pc in enumerate(fl):
                per[(j * (32 - LAG)) // len(fl)].append(pc)
        jobs = [P(r_part, b, j // 8, j % 8, per[j]) for j in range(32)]
        nk, ng = 11, 5
        for mc in range(2):
            if b == 0 and mc == 1:
                wkt[1] = make_w_ops(1)
            j0 = mc * (nk + ng)
            kj = jobs[j0:j0 + nk]
            kt = proj(wkt[mc], b, Weave(kj, 49))
            if b == 0 and mc == 0:
                xcopy(1).wait()
                for bb in range(2, NB):
                    xcopy(bb).start()
                c_wq.start()
                c_wo.start()
                c_wv.start()
            elif b >= 1 or mc == 1:
                for _ in range(min(len(late), 10)):
                    late.pop(0).start()
            pk = {k: _phi(v) for k, v in kt.items()}
            for c in range(4):
                zs = (pk[(0, c)] + pk[(1, c)]) + (pk[(2, c)] + pk[(3, c)])
                z_acc[(c, mc)] = zs if b == 0 else z_acc[(c, mc)] + zs
            pblocks = {(c, r): pk[(r, c)] for r in range(4) for c in range(4)}
            p_ops = [o.astype(bf16) for o in st_ops(pblocks, 2, UA)]
            weave = Weave(jobs[j0 + nk:j0 + nk + ng], 98)
            for n in range(2):
                def prod(p):
                    return weave(_dot(p_ops[p], s_ops[b][PI[p // 7] * 7 + PI[p % 7]][:, n * 128:(n + 1) * 128]))
                g = st_combine(prod, 2)
                for k, v in g.items():
                    kk = (k, mc, n)
                    g_acc[kk] = v if b == 0 else g_acc[kk] + v

    for c in late:
        c.start()
    kf = best["k"]
    for sh in (64, 32, 16, 8, 4, 2, 1):
        kf = jnp.maximum(kf, pltpu.roll(kf, sh, 1))
    kb = kf & (-65536)
    kb = kb ^ ((kb >> 31) & 0x7FFFFFFF)
    key_v = pltpu.bitcast(kb & (-65536), f32)[0:1, 0:1]
    r_sel = jnp.where(key_v == -jnp.inf, best["row0"], key_v)
    idx = jnp.clip(jnp.max((65535 - (kf & 65535))[0:1, :].astype(f32)).astype(i32), 0, S - 1)
    base16 = pl.multiple_of((idx // 16) * 16, 16)
    sel = (lax.broadcasted_iota(i32, (16, 128), 0) + base16) == idx
    xs = jnp.concatenate([jnp.where(sel, xn_t[t, pl.ds(base16, 16), :].astype(f32), 0.0).astype(bf16)
                          for t in range(8)], axis=1)
    ffn = {}

    def ffn_gu(n):
        g = _dot(xs, _b16(wg_v.bitcast(u32)[n]))
        u = _dot(xs, _b16(wu_v.bitcast(u32)[n]))
        ffn[("h", n)] = (g * jax.nn.sigmoid(g) * u).astype(bf16)

    def ffn_down(n, kc):
        hh = jnp.concatenate([ffn[("h", j)] for j in range(7 * kc, 7 * kc + 7)], axis=1)
        d = _dot(hh, _b16(wd_v.bitcast(u32)[n, pl.ds(kc * 448, 448), :]))
        ffn[("y", n)] = d if kc == 0 else ffn[("y", n)] + d
        if kc == 3:
            y = ffn[("y", n)] * jax.nn.sigmoid(r_sel)
            old = xn_t[n, pl.ds(base16, 16), :].astype(f32)
            xn_t[n, pl.ds(base16, 16), :] = (old + jnp.where(sel, y, 0.0)).astype(bf16)

    fgu = split([P(ffn_gu, n) for n in range(NF)], 2)
    fdn = [P(ffn_down, n, kc) for kc in range(4) for n in range(8)]

    zb = {k: jnp.broadcast_to(_rnd(jnp.sum(v, axis=1, keepdims=True)), (128, 128)) for k, v in z_acc.items()}
    ri = lax.broadcasted_iota(i32, (128, 128), 0) // DH
    ci_ = lax.broadcasted_iota(i32, (128, 128), 1) // DH
    bd = ri == ci_

    wqt = [None, None]
    mt_ops = [None, None]

    def q_chunk(b, mc, pieces):
        qt = proj(wqt[mc], b, Weave(pieces, 49))
        pqn = {}
        for (r, c), v in qt.items():
            pq = _phi(v)
            t = (pq * zb[(c, mc)]).reshape(4, DH, 128)
            den = jnp.sum(t, axis=1, keepdims=True) + 1e-6
            pqn[(r, c)] = (pq.reshape(4, DH, 128) * _rcp(den)).reshape(128, 128)
        return pqn

    def o_chunk(b, mo, q_ops):
        def prod(p):
            return _dot(mt_ops[mo][p], q_ops[p])
        at = st_combine(prod, 2)
        for (r, c), v in at.items():
            r0 = b * BT + r * TQ
            c0 = c * FQ + mo * 128
            xx = x_v[r0:r0 + TQ, c0:c0 + 128].astype(f32)
            xn = xn_t[2 * c + mo, r0:r0 + TQ, :].astype(f32)
            o_v[b][r * TQ:(r + 1) * TQ, c0:c0 + 128] = ((xx + v.T) + xn).astype(bf16)

    def q_ops_of(parts):
        per = [[o.astype(bf16) for o in st_ops(pq, 2, UA)] for pq in parts]
        return [jnp.concatenate([per[0][p], per[1][p]], axis=0) for p in range(49)]

    with scope("M"):
        wqt[0] = make_w_ops(0)
        pq00 = q_chunk(0, 0, [])
        kvs = []
        for j in range(8):
            r, mc = j // 2, j % 2
            lhs = jnp.concatenate([g_acc[((r, c), mc, n)].astype(bf16) for c in range(4) for n in range(2)], axis=1)
            kvj = _dot(lhs, wv_v[:, j * 128:(j + 1) * 128])
            kvs.append(jnp.where(bd, kvj, 0.0).astype(bf16))
        wqt[1] = make_w_ops(1)
        pq01 = q_chunk(0, 1, [])
        for c in c_wg + c_wu + c_wd:
            c.wait()
        wu_ = wot_v.bitcast(u32)
        mt = [_dot_nt(_b16(wu_[j]), kvs[j]) for j in range(8)]
        pq10 = q_chunk(1, 0, fgu[0])
        for mo in range(2):
            blocks = {}
            for r in range(4):
                for c in range(4):
                    r0 = c * FQ + mo * 128
                    blocks[(r, c)] = jnp.concatenate([mt[2 * r][r0:r0 + 128, :], mt[2 * r + 1][r0:r0 + 128, :]], axis=1)
            mt_ops[mo] = [o.astype(bf16) for o in st_ops(blocks, 2, UB)]
        pq11 = q_chunk(1, 1, fgu[1] + fdn)
    pq = {0: [pq00, pq01], 1: [pq10, pq11]}
    for b in range(NB):
      with scope("B%d" % b):
        q_ops = q_ops_of(pq.pop(b))
        o_chunk(b, 0, q_ops)
        if b + 2 < NB:
            pq[b + 2] = [q_chunk(b + 2, 0, [])]
        o_chunk(b, 1, q_ops)
        ocopy(b).start()
        if b + 2 < NB:
            pq[b + 2].append(q_chunk(b + 2, 1, []))
    for b in range(NB):
        ocopy(b).wait()


def _w128(*lead):
    return pltpu.VMEM(tuple(lead) + (128,), bf16)


@jax.jit
def pallas_parallel_sum__linear_attn_block__moe_arch_mod__prompt_kernel(
        A_x, A_wqkv, A_wo, B_x, B_w_r, B_w_gate, B_w_up, B_w_down):
    del B_x
    any_spec = pl.BlockSpec(memory_space=pl.ANY)
    ops = _w128(49, 2, 128)
    scratch = (
        [pltpu.VMEM((S, D), bf16)] + [pltpu.VMEM((D, D), bf16)] * 4
        + [pltpu.VMEM((D,), bf16), _w128(F // 128, D), _w128(F // 128, D), _w128(8, F)]
        + [pltpu.VMEM((BT, D), bf16)] * NB
        + [_w128(8, S), _w128(8, D)]
        + [pltpu.VMEM((32, 128, 128), f32)] * 2
        + [pltpu.SemaphoreType.DMA((NB + 4,)), pltpu.SemaphoreType.DMA((16,)), pltpu.SemaphoreType.DMA((NB,)),
           pltpu.SemaphoreType.DMA((F // 128,)), pltpu.SemaphoreType.DMA((F // 128,)), pltpu.SemaphoreType.DMA((8,))]
    )
    return pl.pallas_call(
        kernel,
        out_shape=jax.ShapeDtypeStruct((1, S, D), bf16),
        in_specs=[any_spec] * 7,
        out_specs=any_spec,
        scratch_shapes=scratch,
        compiler_params=pltpu.CompilerParams(vmem_limit_bytes=124 * 1024 * 1024),
        name="psum_la_mod",
    )(A_x, A_wqkv, A_wo, B_w_r, B_w_gate, B_w_up, B_w_down)
```

```python
import functools
import numpy as np
import jax
import jax.numpy as jnp
from jax import lax
import jax.experimental.pallas as pl
import jax.experimental.pallas.tpu as pltpu

S, D, F, H, DH = 2048, 1024, 3584, 32, 32
BT = 512
NB = S // BT
TQ = BT // 4
FQ = D // 4
MCK = 256
MCQ = 256
MCG = 256
MO = 128
f32, bf16, i32, u32 = jnp.float32, jnp.bfloat16, jnp.int32, jnp.uint32
CH = 128
NH = 128 // CH
LAG = 2
KSPAN = 0.95

UA = [{0: 1, 3: 1}, {2: 1, 3: 1}, {0: 1}, {3: 1}, {0: 1, 1: 1}, {2: 1, 0: -1}, {1: 1, 3: -1}]
UB = [{0: 1, 3: 1}, {0: 1}, {1: 1, 3: -1}, {2: 1, 0: -1}, {3: 1}, {0: 1, 1: 1}, {2: 1, 3: 1}]
WC = {0: {0: 1, 3: 1, 4: -1, 6: 1}, 1: {2: 1, 4: 1}, 2: {1: 1, 3: 1}, 3: {0: 1, 1: -1, 2: 1, 5: 1}}
PI = [0, 2, 6, 5, 3, 4, 1]
PORDER = [2, 4, 1, 3, 0, 6, 5]


def _lin(terms):
    acc = None
    for s, v in terms:
        if acc is None:
            acc = v if s > 0 else -v
        else:
            acc = acc + v if s > 0 else acc - v
    return acc


def st_ops(blocks, lvl, U):
    if lvl == 0:
        return [blocks[(0, 0)]]
    h = 2 ** (lvl - 1)
    quad = {q: {(r, c): blocks[(r + (q // 2) * h, c + (q % 2) * h)] for r in range(h) for c in range(h)}
            for q in range(4)}
    out = []
    for u in U:
        sub = {(r, c): _lin([(s, quad[q][(r, c)]) for q, s in sorted(u.items(), key=lambda t: -t[1])])
               for r in range(h) for c in range(h)}
        out += st_ops(sub, lvl - 1, U)
    return out


def st_combine(getp, lvl, base=0):
    if lvl == 0:
        return {(0, 0): getp(base)}
    h = 2 ** (lvl - 1)
    acc = {q: None for q in range(4)}
    for p in PORDER:
        m = st_combine(getp, lvl - 1, base * 7 + p)
        for q in range(4):
            if p in WC[q]:
                s = WC[q][p]
                if acc[q] is None:
                    acc[q] = (s, m)
                else:
                    s0, a = acc[q]
                    if s0 > 0:
                        acc[q] = (1, {k: (a[k] + m[k] if s > 0 else a[k] - m[k]) for k in m})
                    else:
                        assert s > 0
                        acc[q] = (1, {k: m[k] - a[k] for k in m})
    res = {}
    for q in range(4):
        assert acc[q][0] > 0
        for (r, c), v in acc[q][1].items():
            res[(r + (q // 2) * h, c + (q % 2) * h)] = v
    return res


def _dot(a, b):
    return jnp.dot(a, b, preferred_element_type=f32)


def _dot_nt(a, b):
    return lax.dot_general(a, b, (((1,), (1,)), ((), ())), preferred_element_type=f32)


def _phi(t):
    return jnp.where(t > 0, t + 1.0, jnp.exp(t)) + 1e-6


def _rnd(t):
    return t.astype(bf16).astype(f32)


def _rsum(v):
    return jnp.broadcast_to(jnp.sum(v, axis=1, keepdims=True), (v.shape[0], 128))


def _rcp(t):
    return pltpu.reciprocal(t, approx=False, full_range=False)


def _tiles(v):
    return [v[:, t * 128:(t + 1) * 128] for t in range(v.shape[1] // 128)]


def _layernorm_tiles(xt):
    mean = _rsum(functools.reduce(lambda a, b: a + b, xt)) * (1.0 / D)
    var = _rsum(functools.reduce(lambda a, b: a + b, [(t - mean) * (t - mean) for t in xt])) * (1.0 / D)
    m_b = _rnd(mean)
    s_b = _rnd(jnp.sqrt(_rnd(_rnd(var) + EPS_B)))
    rs = _rcp(s_b)
    return [(t - m_b) * rs for t in xt]


import contextlib
scope = lambda n: contextlib.nullcontext()
EPS_B = float(np.float32(1.0013580322265625e-05))


def _b16(v):
    return pltpu.bitcast(v, bf16)


def kernel(x_hbm, wqkv_hbm, wo_hbm, wr_hbm, wg_hbm, wu_hbm, wd_hbm, o_hbm, *scr):
    it = iter(scr)
    take = lambda n: [next(it) for _ in range(n)]
    x_v, wq_v, wk_v, wv_v, wo_v, wr_v, wg_v, wu_v, wd_v = take(9)
    o_v = take(NB)
    xn_t, wot_v = take(2)
    wt_v = take(2)
    sem_x, sem_w, sem_o, sem_g, sem_u, sem_d = take(6)
    NF = F // 128
    FG = 4

    def xcopy(b):
        return pltpu.make_async_copy(x_hbm.at[0, pl.ds(b * BT, BT)], x_v.at[pl.ds(b * BT, BT)], sem_x.at[b])

    def ocopy(b):
        return pltpu.make_async_copy(o_v[b], o_hbm.at[0, pl.ds(b * BT, BT)], sem_o.at[b])

    def wk_copy(m, c):
        return pltpu.make_async_copy(wqkv_hbm.at[:, pl.ds(D + c * FQ + m * 128, 128)],
                                     wk_v.at[:, pl.ds(c * FQ + m * 128, 128)], sem_w.at[8 + m * 4 + c])

    c_wr = pltpu.make_async_copy(wr_hbm, wr_v, sem_w.at[0])
    c_wv = pltpu.make_async_copy(wqkv_hbm.at[:, pl.ds(2 * D, D)], wv_v, sem_w.at[2])
    c_wo = pltpu.make_async_copy(wo_hbm, wo_v, sem_w.at[3])
    c_wq = pltpu.make_async_copy(wqkv_hbm.at[:, pl.ds(0, D)], wq_v, sem_w.at[4])
    c_wg = [pltpu.make_async_copy(wg_hbm.at[:, pl.ds(n * 128, 128)], wg_v.at[n], sem_g.at[n]) for n in range(NF)]
    c_wu = [pltpu.make_async_copy(wu_hbm.at[:, pl.ds(n * 128, 128)], wu_v.at[n], sem_u.at[n]) for n in range(NF)]
    c_wd = [pltpu.make_async_copy(wd_hbm.at[:, pl.ds(n * 128, 128)], wd_v.at[n], sem_d.at[n]) for n in range(8)]
    c_x0 = [pltpu.make_async_copy(x_hbm.at[0, pl.ds(q * TQ, TQ)], x_v.at[pl.ds(q * TQ, TQ)], sem_x.at[NB + q])
            for q in range(4)]
    c_x0[0].start()
    c_wr.start()
    c_x0[1].start()

    def start_ffn_copies():
        for c in c_wd:
            c.start()
        for n in range(NF):
            c_wg[n].start()
            c_wu[n].start()

    late = list(c_wd)
    for n in range(NF):
        late += [c_wg[n], c_wu[n]]
    st = {}
    c_wr.wait()
    wr16 = jnp.broadcast_to(wr_v[...].reshape(1, D), (16, D))
    xn_u = xn_t.bitcast(u32)
    stats = {}
    best = {}

    def xl(b, g, t):
        r0 = b * BT + g * 16
        return x_v[r0:r0 + 16, t * 128:(t + 1) * 128].astype(f32)

    def ln_a(b, g):
        s_ = xl(b, g, 0)
        for t in range(1, 8):
            s_ = s_ + xl(b, g, t)
        mean = _rsum(s_) * (1.0 / D)
        stats[("m", b, g)] = mean
        return pltpu.bitcast(mean[8:16, :], u32)

    def ln_b(b, g):
        mean = stats.pop(("m", b, g))
        q = None
        for t in range(8):
            e = xl(b, g, t) - mean
            q = e * e if q is None else q + e * e
        var = _rsum(q) * (1.0 / D)
        m_b = _rnd(mean)
        s_b = _rnd(jnp.sqrt(_rnd(_rnd(var) + EPS_B)))
        rs = _rcp(s_b)
        if "fmask" not in st:
            sb = s_b[0:8, :]
            st["fmask"] = sb < 0.0
            st["z"] = [jnp.max(jnp.where(sb < -float(k), 1.0, 0.0)).astype(i32) for k in range(2)]
        stats[(b, g)] = (m_b, rs)
        return pltpu.bitcast(rs[8:16, :], u32)

    def ln_c(b, g):
        r0 = b * BT + g * 16
        m_b, rs = stats.pop((b, g))
        for t in range(8):
            xn_t[t, r0:r0 + 16, :] = ((xl(b, g, t) - m_b) * rs).astype(bf16)

    def r_part(b, tt, t, pieces):
        t0 = b * BT + tt * 128
        ru = xn_u[t, pl.ds(t0 // 2, 64), :]
        k = 0
        for fn, buf in pieces:
            tok = fn()
            pend.append((len(hosted) + LAG, tok if buf is None else anchor(buf)))
        hosted.append(0)
        last = tt == 3 and t == 7
        while pend and (last or pend[0][0] <= len(hosted)):
            tok = pend.pop(0)[1]
            hd = jnp.where(st["fmask"], tok, ru[8 * k:8 * k + 8, :])
            ru = jnp.concatenate(([ru[:8 * k, :]] if k else []) + [hd] + ([ru[8 * k + 8:, :]] if k < 7 else []), axis=0)
            k = min(k + 1, 7)
        d = _dot_nt(wr16[:, t * 128:(t + 1) * 128], _b16(ru))[0:8, :]
        acc = d if t == 0 else racc.pop() + d
        if t < 7:
            racc.append(acc)
            return
        rr = _rnd(acc)
        if t0 == 0:
            best["row0"] = rr[0:1, 0:1]
        kb = pltpu.bitcast(jnp.where(rr == rr, rr, -jnp.inf), i32)
        kb = kb ^ ((kb >> 31) & 0x7FFFFFFF)
        kb = (kb & (-65536)) | (65535 - t0 - lax.broadcasted_iota(i32, (8, 128), 1))
        best["k"] = kb if "k" not in best else jnp.maximum(best["k"], kb)

    pend = []
    hosted = []
    racc = []

    def wt_piece(w_ref, m, r, c):
        for kt in range(2):
            t = w_ref[r * FQ + kt * 128:r * FQ + (kt + 1) * 128, c * FQ + m * 128:c * FQ + (m + 1) * 128]
            wt_v[m][(r * 4 + c) * 2 + kt] = t.astype(f32).T

    def wot_piece(j, t):
        v = wo_v[j * 128:(j + 1) * 128, t * 128:(t + 1) * 128].astype(f32).T
        wot_v[j, t * 128:(t + 1) * 128, :] = v.astype(bf16)

    def anchor(buf):
        idx = (st["z"][1],) + (0,) * (len(buf.shape) - 3) + (pl.ds(0, 8), pl.ds(0, 128))
        if buf.dtype == bf16:
            return buf.bitcast(u32)[idx]
        return pltpu.bitcast(buf[idx], u32)

    class Weave:
        def __init__(self, jobs, nslots):
            self.i = 0
            self.todo = [((j * nslots) // len(jobs), fn) for j, fn in enumerate(jobs)] if jobs else []

        def __call__(self, v):
            while self.todo and self.todo[0][0] <= self.i:
                self.todo.pop(0)[1]()
            self.i += 1
            return v

    P = functools.partial

    def f_ln(b):
        out = []
        for j in range(34):
            if j < 32:
                out.append((P(ln_a, b, j), None))
            if 1 <= j < 33:
                out.append((P(ln_b, b, j - 1), None))
            if j >= 2:
                out.append((P(ln_c, b, j - 2), xn_t))
        return out

    def f_wt(w_ref, m):
        return [(P(wt_piece, w_ref, m, r, c), wt_v[m]) for c in range(4) for r in range(4)]

    def split(lst, n):
        return [lst[i * len(lst) // n:(i + 1) * len(lst) // n] for i in range(n)]

    def make_w_ops(m, h):
        per = [[o.astype(bf16) for o in st_ops({(r, c): wt_v[m][(r * 4 + c) * 2 + kt, h * CH:(h + 1) * CH, :]
                                                for r in range(4) for c in range(4)}, 2, UB)] for kt in range(2)]
        return [[per[0][p], per[1][p]] for p in range(49)]

    s_ops = [None] * NB

    def make_s_ops(b):
        per = [[o.astype(bf16) for o in st_ops({(r, c): xn_t[2 * c + kt, b * BT + r * TQ:b * BT + (r + 1) * TQ, :].astype(f32)
                                                for r in range(4) for c in range(4)}, 2, UA)] for kt in range(2)]
        s_ops[b] = [[per[0][p], per[1][p]] for p in range(49)]

    def proj(wops, b, weave):
        return st_combine(lambda p: weave(_dot_nt(wops[p][0], s_ops[b][p][0]) + _dot_nt(wops[p][1], s_ops[b][p][1])), 2)

    for q in range(4):
        c_x0[q].wait()
        if q < 2:
            c_x0[q + 2].start()
        else:
            wk_copy(0, 2 * q - 4).start()
            wk_copy(0, 2 * q - 3).start()
        for g in range(8 * q, 8 * q + 8):
            ln_a(0, g)
        for g in range(8 * q, 8 * q + 8):
            ln_b(0, g)
        for g in range(8 * q, 8 * q + 8):
            ln_c(0, g)
    for c in range(4):
        wk_copy(0, c).wait()
        wk_copy(1, c).start()
        for r in range(4):
            wt_piece(wk_v, 0, r, c)
    for c in range(4):
        wk_copy(1, c).wait()
    xcopy(1).start()
    wkt = {(0, 0): make_w_ops(0, 0)}

    g_acc = {}
    z_acc = {}
    for b in range(NB):
      with scope("A%d" % b):
        if 1 <= b < NB - 1:
            xcopy(b + 1).wait()
        if b == NB - 1:
            c_wq.wait()
            c_wo.wait()
            c_wv.wait()
        make_s_ops(b)
        if b + 1 < NB:
            lnp = f_ln(b + 1)
            per = [[] for _ in range(32)]
            first = (32 // (4 * NH)) * 2 + 2 if b == 0 else 0
            for j, pc in enumerate(lnp):
                per[first + (j * (32 - first - LAG)) // len(lnp)].append(pc)
            if b == 0:
                for j, pc in enumerate(f_wt(wk_v, 1)):
                    per[j // 4].append(pc)
        else:
            fl = f_wt(wq_v, 0) + f_wt(wq_v, 1) + [(P(wot_piece, j, t), wot_v) for j in range(8) for t in range(8)]
            per = [[] for _ in range(32)]
            for j, pc in enumerate(fl):
                per[(j * (32 - LAG)) // len(fl)].append(pc)
        jobs = [P(r_part, b, j // 8, j % 8, per[j]) for j in range(32)]
        nq = 2 * NH
        kj = split(jobs, 2 * nq)
        for ci in range(nq):
            mc, h = ci // NH, ci % NH
            if (mc, h) not in wkt:
                wkt[(mc, h)] = make_w_ops(mc, h)
            kt = proj(wkt[(mc, h)], b, Weave(kj[2 * ci], 49))
            if b == 0 and ci == 0:
                xcopy(1).wait()
                for bb in range(2, NB):
                    xcopy(bb).start()
                c_wq.start()
                c_wo.start()
                c_wv.start()
            elif ci % NH == 0:
                for _ in range(min(len(late), 10)):
                    late.pop(0).start()
            pk = {k: _phi(v) for k, v in kt.items()}
            for c in range(4):
                zs = (pk[(0, c)] + pk[(1, c)]) + (pk[(2, c)] + pk[(3, c)])
                z_acc[(c, ci)] = zs if b == 0 else z_acc[(c, ci)] + zs
            pblocks = {(c, r): pk[(r, c)] for r in range(4) for c in range(4)}
            p_ops = [o.astype(bf16) for o in st_ops(pblocks, 2, UA)]
            weave = Weave(kj[2 * ci + 1], 98)
            for n in range(2):
                def prod(p):
                    return weave(_dot(p_ops[p], s_ops[b][PI[p // 7] * 7 + PI[p % 7]][n]))
                g = st_combine(prod, 2)
                for k, v in g.items():
                    kk = (k, ci, n)
                    g_acc[kk] = v if b == 0 else g_acc[kk] + v

    for c in late:
        c.start()
    kf = best["k"]
    for sh in (64, 32, 16, 8, 4, 2, 1):
        kf = jnp.maximum(kf, pltpu.roll(kf, sh, 1))
    kb = kf & (-65536)
    kb = kb ^ ((kb >> 31) & 0x7FFFFFFF)
    key_v = pltpu.bitcast(kb & (-65536), f32)[0:1, 0:1]
    r_sel = jnp.where(key_v == -jnp.inf, best["row0"], key_v)
    idx = jnp.clip(jnp.max((65535 - (kf & 65535))[0:1, :].astype(f32)).astype(i32), 0, S - 1)
    base16 = pl.multiple_of((idx // 16) * 16, 16)
    sel = (lax.broadcasted_iota(i32, (16, 128), 0) + base16) == idx
    xs = jnp.concatenate([jnp.where(sel, xn_t[t, pl.ds(base16, 16), :].astype(f32), 0.0).astype(bf16)
                          for t in range(8)], axis=1)
    ffn = {}

    def ffn_gu(n):
        g = _dot(xs, _b16(wg_v.bitcast(u32)[n]))
        u = _dot(xs, _b16(wu_v.bitcast(u32)[n]))
        ffn[("h", n)] = (g * jax.nn.sigmoid(g) * u).astype(bf16)

    def ffn_down(n, kc):
        hh = jnp.concatenate([ffn[("h", j)] for j in range(7 * kc, 7 * kc + 7)], axis=1)
        d = _dot(hh, _b16(wd_v.bitcast(u32)[n, pl.ds(kc * 448, 448), :]))
        ffn[("y", n)] = d if kc == 0 else ffn[("y", n)] + d
        if kc == 3:
            y = ffn[("y", n)] * jax.nn.sigmoid(r_sel)
            old = xn_t[n, pl.ds(base16, 16), :].astype(f32)
            xn_t[n, pl.ds(base16, 16), :] = (old + jnp.where(sel, y, 0.0)).astype(bf16)

    fgu = split([P(ffn_gu, n) for n in range(NF)], 2)
    fdn = [P(ffn_down, n, kc) for kc in range(4) for n in range(8)]

    zb = {k: jnp.broadcast_to(_rnd(jnp.sum(v, axis=1, keepdims=True)), (CH, 128)) for k, v in z_acc.items()}
    ri = lax.broadcasted_iota(i32, (128, 128), 0) // DH
    ci_ = lax.broadcasted_iota(i32, (128, 128), 1) // DH
    bd = ri == ci_

    wqt = {}
    mt_ops = [None, None]

    def q_chunk(b, mc, pieces):
        halves = []
        pcs = split(pieces, NH)
        for h in range(NH):
            if (mc, h) not in wqt:
                wqt[(mc, h)] = make_w_ops(mc, h)
            qt = proj(wqt[(mc, h)], b, Weave(pcs[h], 49))
            pqn = {}
            for (r, c), v in qt.items():
                pq = _phi(v)
                t = (pq * zb[(c, mc * NH + h)]).reshape(CH // DH, DH, 128)
                den = jnp.sum(t, axis=1, keepdims=True) + 1e-6
                pqn[(r, c)] = (pq.reshape(CH // DH, DH, 128) * _rcp(den)).reshape(CH, 128)
            halves.append(pqn)
        return {k: jnp.concatenate([hv[k] for hv in halves], axis=0) for k in halves[0]}

    def o_chunk(b, mo, q_ops):
        def prod(p):
            return _dot(mt_ops[mo][p][0], q_ops[p][0]) + _dot(mt_ops[mo][p][1], q_ops[p][1])
        at = st_combine(prod, 2)
        for (r, c), v in at.items():
            r0 = b * BT + r * TQ
            c0 = c * FQ + mo * 128
            xx = x_v[r0:r0 + TQ, c0:c0 + 128].astype(f32)
            xn = xn_t[2 * c + mo, r0:r0 + TQ, :].astype(f32)
            o_v[b][r * TQ:(r + 1) * TQ, c0:c0 + 128] = ((xx + v.T) + xn).astype(bf16)

    def q_ops_of(parts):
        per = [[o.astype(bf16) for o in st_ops(pq, 2, UA)] for pq in parts]
        return [[per[0][p], per[1][p]] for p in range(49)]

    fall = [fgu[0][:11], fgu[0][11:] + fgu[1][:8], fgu[1][8:] + fdn[:8], fdn[8:]]
    with scope("M"):
        pq00 = q_chunk(0, 0, [])
        kvs = []
        for j in range(8):
            r, mc = j // 2, j % 2
            kvj = functools.reduce(lambda a, b_: a + b_, [
                _dot(jnp.concatenate([g_acc[((r, c), mc * NH + h, n)] for h in range(NH)], axis=0).astype(bf16),
                     wv_v[(2 * c + n) * 128:(2 * c + n + 1) * 128, j * 128:(j + 1) * 128])
                for c in range(4) for n in range(2)])
            kvs.append(jnp.where(bd, kvj, 0.0).astype(bf16))
        pq01 = q_chunk(0, 1, [])
        for c in c_wg + c_wu + c_wd:
            c.wait()
        wu_ = wot_v.bitcast(u32)
        mt = [_dot_nt(_b16(wu_[j]), kvs[j]) for j in range(8)]
        pq10 = q_chunk(1, 0, fall[0])
        for mo in range(2):
            blocks = {}
            for r in range(4):
                for c in range(4):
                    r0 = c * FQ + mo * 128
                    for kt in range(2):
                        blocks[(kt, r, c)] = mt[2 * r + kt][r0:r0 + 128, :]
            per = [[o.astype(bf16) for o in st_ops({(r, c): blocks[(kt, r, c)] for r in range(4) for c in range(4)}, 2, UB)]
                   for kt in range(2)]
            mt_ops[mo] = [[per[0][p], per[1][p]] for p in range(49)]
        pq11 = q_chunk(1, 1, fall[1])
        pq2 = [q_chunk(2, 0, fall[2]), q_chunk(2, 1, fall[3])]
    pq = {0: [pq00, pq01], 1: [pq10, pq11], 2: pq2}
    for b in range(NB):
      with scope("B%d" % b):
        q_ops = q_ops_of(pq.pop(b))
        o_chunk(b, 0, q_ops)
        if b + 3 < NB:
            pq[b + 3] = [q_chunk(b + 3, 0, [])]
        o_chunk(b, 1, q_ops)
        ocopy(b).start()
        if b + 3 < NB:
            pq[b + 3].append(q_chunk(b + 3, 1, []))
    for b in range(NB):
        ocopy(b).wait()


def _w128(*lead):
    return pltpu.VMEM(tuple(lead) + (128,), bf16)


@jax.jit
def pallas_parallel_sum__linear_attn_block__moe_arch_mod__prompt_kernel(
        A_x, A_wqkv, A_wo, B_x, B_w_r, B_w_gate, B_w_up, B_w_down):
    del B_x
    any_spec = pl.BlockSpec(memory_space=pl.ANY)
    ops = _w128(49, 2, 128)
    scratch = (
        [pltpu.VMEM((S, D), bf16)] + [pltpu.VMEM((D, D), bf16)] * 4
        + [pltpu.VMEM((D,), bf16), _w128(F // 128, D), _w128(F // 128, D), _w128(8, F)]
        + [pltpu.VMEM((BT, D), bf16)] * NB
        + [_w128(8, S), _w128(8, D)]
        + [pltpu.VMEM((32, 128, 128), f32)] * 2
        + [pltpu.SemaphoreType.DMA((NB + 4,)), pltpu.SemaphoreType.DMA((16,)), pltpu.SemaphoreType.DMA((NB,)),
           pltpu.SemaphoreType.DMA((F // 128,)), pltpu.SemaphoreType.DMA((F // 128,)), pltpu.SemaphoreType.DMA((8,))]
    )
    return pl.pallas_call(
        kernel,
        out_shape=jax.ShapeDtypeStruct((1, S, D), bf16),
        in_specs=[any_spec] * 7,
        out_specs=any_spec,
        scratch_shapes=scratch,
        compiler_params=pltpu.CompilerParams(vmem_limit_bytes=124 * 1024 * 1024),
        name="psum_la_mod",
    )(A_x, A_wqkv, A_wo, B_w_r, B_w_gate, B_w_up, B_w_down)
```
